```python
import os as _os
_os.environ.setdefault("JAX_PLATFORMS", "cpu")
import jax
import jax.numpy as jnp

def _softmax(x, axis=-1):
    return jax.nn.softmax(x, axis=axis)
def _gelu(x):
    return jax.nn.gelu(x, approximate=True)
def _silu(x):
    return jax.nn.silu(x)
def _sigmoid(x):
    return jax.nn.sigmoid(x)
def _layernorm(x, axis=-1, eps=1e-5):
    m = jnp.mean(x, axis=axis, keepdims=True)
    v = jnp.var(x, axis=axis, keepdims=True)
    return (x - m) / jnp.sqrt(v + eps)
def _scatter_add(tgt, idx, src, axis=0):
    return tgt.at[idx].add(src)
def _segment_sum(src, seg, n):
    return jax.ops.segment_sum(src, seg, n)
class _Rng:
    def __init__(self, key):
        self._k = key
    def _next(self):
        self._k, sub = jax.random.split(self._k)
        return sub
    def normal(self, shape):
        return jax.random.normal(self._next(), shape, dtype=jnp.bfloat16)
    def randint(self, lo, hi, shape):
        return jax.random.randint(self._next(), shape, lo, hi, dtype=jnp.int32)
    def uniform(self, shape, lo=0.0, hi=1.0):
        return jax.random.uniform(self._next(), shape, jnp.bfloat16, lo, hi)
    def permutation(self, n):
        return jax.random.permutation(self._next(), n)


kernel_name = 'parallel_sum__ssm_conv_s4__mixer_channel_mlp__prompt'

def setup_inputs():
    _rng = _Rng(jax.random.key(int.from_bytes(__import__("os").urandom(4), "little")))
    _w = (lambda a: (lambda t: t.astype(jnp.bfloat16) if jnp.issubdtype(t.dtype, jnp.floating) else t)(jnp.asarray(a)))
    def _A_setup():
        B, L, D, N = 1, 2048, 512, 128
        A_re = -jnp.exp((lambda *s: _rng.normal(s) * 0.1)(D, N))
        A_im = jnp.pi * (lambda *s: _rng.normal(s) * 0.1)(D, N)
        B_re = (lambda *s: _rng.normal(s) * 0.1)(D, N)
        B_im = (lambda *s: _rng.normal(s) * 0.1)(D, N)
        C_re = (lambda *s: _rng.normal(s) * 0.1)(D, N)
        C_im = (lambda *s: _rng.normal(s) * 0.1)(D, N)
        log_dt = (lambda *s: _rng.normal(s) * 0.1)(D) * 0.5 - 4.0
        Dskip = (lambda *s: _rng.normal(s) * 0.05)(D)
        return {
            "u": _w((lambda *s: _rng.normal(s) * 0.05)(B, L, D)),
            "A_re": _w(A_re),
            "A_im": _w(A_im),
            "B_re": _w(B_re),
            "B_im": _w(B_im),
            "C_re": _w(C_re),
            "C_im": _w(C_im),
            "log_dt": _w(log_dt),
            "Dskip": _w(Dskip),
        }
    _A_in = _A_setup()

    def _B_setup():
        B, S, D, F = 1, 2048, 512, 1792
        return {
            "x": _w((lambda *s: _rng.normal(s) * 0.05)(B, S, D)),
            "w1": _w((lambda *s: _rng.normal(s) * 0.2)(D, F) * (D ** -0.5)),
            "b1": _w((lambda *s: _rng.normal(s) * 0.2)(F)),
            "w2": _w((lambda *s: _rng.normal(s) * 0.2)(F, D) * (F ** -0.5)),
            "b2": _w((lambda *s: _rng.normal(s) * 0.05)(D)),
        }
    _B_in = _B_setup()

    return {
        "A_u": _A_in["u"],
        "A_A_re": _A_in["A_re"],
        "A_A_im": _A_in["A_im"],
        "A_B_re": _A_in["B_re"],
        "A_B_im": _A_in["B_im"],
        "A_C_re": _A_in["C_re"],
        "A_C_im": _A_in["C_im"],
        "A_log_dt": _A_in["log_dt"],
        "A_Dskip": _A_in["Dskip"],
        "B_x": _B_in["x"],
        "B_w1": _B_in["w1"],
        "B_b1": _B_in["b1"],
        "B_w2": _B_in["w2"],
        "B_b2": _B_in["b2"],
    }

def reference(A_u, A_A_re, A_A_im, A_B_re, A_B_im, A_C_re, A_C_im, A_log_dt, A_Dskip, B_x, B_w1, B_b1, B_w2, B_b2):
    def _A_ref(u, A_re, A_im, B_re, B_im, C_re, C_im, log_dt, Dskip):
        Bsz, L, D = u.shape
        dt = jnp.exp(log_dt)[:, None]
        A = A_re + 1j * A_im
        Bc = B_re + 1j * B_im
        Cc = C_re + 1j * C_im
        logdA = dt * A
        dB = dt * Bc
        l = (lambda x, dt: x.astype(dt))(jnp.arange(L), A_re.dtype)
        P = jnp.exp(logdA[:, :, None] * l[None, None, :])
        K = jnp.einsum("dn,dnl,dn->dl", Cc, P, dB).real
        L2 = 2 * L
        Kp = jnp.pad(K, ((0, 0), (0, L)))
        up = (lambda x, *d: x.transpose(*d))(u, 0, 2, 1)
        up = jnp.pad(up, ((0, 0), (0, 0), (0, L)))
        Kf = (lambda x, axes=(-2,-1): jnp.fft.rfft2(x.astype(jnp.float32), axes=axes))(Kp[:, None, :], axes=(-2, -1))
        Uf = (lambda x, axes=(-2,-1): jnp.fft.rfft2(x.astype(jnp.float32), axes=axes))(up[:, :, None, :], axes=(-2, -1))
        Yf = Uf * Kf[None, :, :, :]
        y = (lambda x, s, axes=(-2,-1): jnp.fft.irfft2(x, s=s, axes=axes).astype(jnp.bfloat16))(Yf, (1, L2), axes=(-2, -1))[:, :, 0, :L]
        y = (lambda x, *d: x.transpose(*d))(y, 0, 2, 1) + u * Dskip[None, None, :]
        return y

    def _B_ref(x, w1, b1, w2, b2):
        y = _layernorm(x, axis=-1)
        h = _gelu(jnp.einsum("bsd,df->bsf", y, w1) + b1)
        return jnp.einsum("bsf,fd->bsd", h, w2) + b2

    x = A_u
    xn = _layernorm(x, axis=-1)
    return x + _A_ref(xn, A_A_re, A_A_im, A_B_re, A_B_im, A_C_re, A_C_im, A_log_dt, A_Dskip) + _B_ref(xn, B_w1, B_b1, B_w2, B_b2)
```

```python
import functools
import numpy as np
import jax
import jax.numpy as jnp
from jax import lax
import jax.experimental.pallas as pl
import jax.experimental.pallas.tpu as pltpu

L, D, N, FF = 2048, 512, 128, 1792
T = 128
NC = L // T


def _dft_consts():
    f = np.concatenate([np.arange(0, 128, 2), np.arange(1, 128, 2)])
    phi = 2 * np.pi * (f + 0.5) / 256
    ang = phi[:, None] * np.arange(128)[None, :]
    F = np.concatenate([np.cos(ang), -np.sin(ang)], 0)
    G = np.concatenate([np.cos(ang).T, -np.sin(ang).T], 1) / 128.0
    return F.astype(np.float32), G.astype(np.float32)

_F_NP, _G_NP = _dft_consts()

f32 = jnp.float32
bf16 = jnp.bfloat16


def cmul(ar, ai, br, bi):
    return ar * br - ai * bi, ar * bi + ai * br


def kernel(x_ref, are_ref, aim_ref, bre_ref, bim_ref, cre_ref, cim_ref, ldt_ref, dsk_ref,
           w1_ref, b1_ref, w2_ref, b2_ref, F_ref, G_ref,
           o_ref,
           pf_ref, pc_ref, m_ref, kt_ref, kf_ref, uf_ref, yf_ref, xn_ref, yl_ref, *, parts):
    dt_row = jnp.exp(ldt_ref[...].astype(f32)).astype(bf16).astype(f32).reshape(1, D)
    dt = jnp.broadcast_to(dt_row, (128, D)).T
    rho = dt * are_ref[...].astype(f32)
    th = dt * aim_ref[...].astype(f32)

    def cexp(k):
        e = jnp.exp(rho * k)
        t = th * k
        return e * jnp.cos(t), e * jnp.sin(t)
    a1 = cexp(1.0)
    a8 = cexp(8.0)
    a64 = cexp(64.0)
    a128 = cexp(128.0)
    a1024 = cexp(1024.0)
    m_ref[0] = a8[0]; m_ref[1] = a8[1]
    m_ref[2] = a64[0]; m_ref[3] = -a64[1]
    m_ref[4] = a1024[0]; m_ref[5] = -a1024[1]
    p = (jnp.ones((D, N), f32), jnp.zeros((D, N), f32))
    for i in range(8):
        pf_ref[0, pl.ds(i * D, D), :] = p[0]
        pf_ref[1, pl.ds(i * D, D), :] = p[1]
        if i < 7:
            p = cmul(p[0], p[1], a1[0], a1[1])
    dbr = dt * bre_ref[...].astype(f32); dbi = dt * bim_ref[...].astype(f32)
    q = cmul(cre_ref[...].astype(f32), cim_ref[...].astype(f32), dbr, dbi)
    for i in range(8):
        pc_ref[0, pl.ds(i * D, D), :] = q[0]
        pc_ref[1, pl.ds(i * D, D), :] = -q[1]
        if i < 7:
            q = cmul(q[0], q[1], a128[0], a128[1])

    lane = lax.broadcasted_iota(jnp.int32, (16, 128), 1)
    lo = lane < 64

    def chan(d):
        def bc(k):
            return jnp.broadcast_to(m_ref[k, pl.ds(d, 1), :], (8, N))
        fr = pf_ref[0, pl.ds(d, 8, stride=D), :]
        fi = pf_ref[1, pl.ds(d, 8, stride=D), :]
        m8r, m8i = bc(0), bc(1)
        frs, fis = [fr], [fi]
        for _ in range(7):
            fr, fi = cmul(fr, fi, m8r, m8i)
            frs.append(fr); fis.append(fi)
        fine_r = jnp.concatenate(frs, 0).astype(bf16)
        fine_i = jnp.concatenate(fis, 0).astype(bf16)
        c0 = (pc_ref[0, pl.ds(d, 8, stride=D), :], pc_ref[1, pl.ds(d, 8, stride=D), :])
        m64 = (bc(2), bc(3)); m1k = (bc(4), bc(5))
        c1 = cmul(*c0, *m1k)
        c2 = cmul(*c0, *m64)
        c3 = cmul(*c2, *m1k)
        co_r = jnp.concatenate([c0[0], c1[0], c2[0], c3[0]], 0).astype(bf16)
        co_i = jnp.concatenate([c0[1], c1[1], c2[1], c3[1]], 0).astype(bf16)
        return fine_r, fine_i, co_r, co_i

    H = D // 2
    UNR = 4

    def kmat_body(it, carry):
        for u in range(UNR):
            p = it * UNR + u
            fa = chan(p); fb = chan(p + H)
            lhs = jnp.concatenate([jnp.concatenate([fa[2], fb[2]], 0), jnp.concatenate([fa[3], fb[3]], 0)], 1)
            rhs = jnp.concatenate([jnp.concatenate([fa[0], fb[0]], 0), jnp.concatenate([fa[1], fb[1]], 0)], 1)
            out = lax.dot_general(lhs, rhs, (((1,), (1,)), ((), ())), preferred_element_type=f32)
            ka = jnp.where(lo, out[0:16], pltpu.roll(out[16:32], 64, 1))
            kb = jnp.where(lo, pltpu.roll(out[32:48], 64, 1), out[48:64])
            kt_ref[pl.ds(p, 16, stride=D), :] = ka
            kt_ref[pl.ds(p + H, 16, stride=D), :] = kb
        return carry
    if 'kmat' in parts:
        lax.fori_loop(0, H // UNR, kmat_body, 0)

    Fm = F_ref[...]
    def dftk_body(j, carry):
        kb = kt_ref[pl.ds(pl.multiple_of(j * D, D), D), :].astype(bf16)
        kf = lax.dot_general(Fm, kb, (((1,), (1,)), ((), ())), preferred_element_type=f32)
        kf_ref[j] = kf
        return carry
    if 'dftk' in parts:
        lax.fori_loop(0, NC, dftk_body, 0)
        def fold_body(i, carry):
            j = NC - 1 - i
            cur = kf_ref[j]; prv = kf_ref[j - 1]
            kf_ref[j, 0:64] = cur[0:64] - prv[128:192]
            kf_ref[j, 64:128] = cur[64:128] + prv[192:256]
            kf_ref[j, 128:192] = cur[128:192] + prv[0:64]
            kf_ref[j, 192:256] = cur[192:256] - prv[64:128]
            return carry
        lax.fori_loop(0, NC - 1, fold_body, 0)

    eps = 1e-5
    def ln_body(c, carry):
        r0 = pl.multiple_of(c * T, T)
        x = x_ref[pl.ds(r0, T), :].astype(f32)
        m = jnp.mean(x, axis=-1, keepdims=True)
        xc = x - m
        v = jnp.mean(xc * xc, axis=-1, keepdims=True)
        xn = xc * lax.rsqrt(v + eps)
        m2 = jnp.mean(xn, axis=-1, keepdims=True)
        x2 = xn - m2
        v2 = jnp.mean(x2 * x2, axis=-1, keepdims=True)
        yl = x2 * lax.rsqrt(v2 + eps)
        xnb = xn.astype(bf16)
        xn_ref[pl.ds(r0, T), :] = xn
        yl_ref[pl.ds(r0, T), :] = yl.astype(bf16)
        uf_ref[c] = jnp.dot(Fm, xnb, preferred_element_type=f32)
        return carry
    if 'ln' in parts:
        lax.fori_loop(0, NC, ln_body, 0)

    def conv_body(pos, carry):
        r = pl.multiple_of((pos // 4) * 8, 8)
        l0 = pl.multiple_of((pos % 4) * 128, 128)
        def ld(ref, i):
            return ref[i, pl.ds(r, 8), pl.ds(l0, 128)], ref[i, pl.ds(r + 128, 8), pl.ds(l0, 128)]
        for cb in range(4):
            cs = list(range(4 * cb, 4 * cb + 4))
            acc = [None] * 4
            kwin = {}
            for cp in range(cs[-1], -1, -1):
                ur, ui = ld(uf_ref, cp)
                for a, c in enumerate(cs):
                    j = c - cp
                    if j < 0:
                        continue
                    if j not in kwin:
                        kwin[j] = ld(kf_ref, j)
                    kr, ki = kwin[j]
                    tr = ur * kr - ui * ki
                    ti = ur * ki + ui * kr
                    acc[a] = (tr, ti) if acc[a] is None else (acc[a][0] + tr, acc[a][1] + ti)
                for j in list(kwin):
                    if j < cs[0] - cp + 1:
                        del kwin[j]
            for a, c in enumerate(cs):
                yf_ref[c, pl.ds(r, 8), pl.ds(l0, 128)] = acc[a][0].astype(yf_ref.dtype)
                yf_ref[c, pl.ds(r + 128, 8), pl.ds(l0, 128)] = acc[a][1].astype(yf_ref.dtype)
        return carry
    if 'conv' in parts:
        lax.fori_loop(0, 64, conv_body, 0)

    dsk = dsk_ref[...].astype(f32).reshape(1, D)
    b1 = b1_ref[...].astype(f32).reshape(1, FF)
    b2 = b2_ref[...].astype(f32).reshape(1, D)
    Gm = G_ref[...]
    TM = 256
    def mlp_body(i, carry):
        r0 = pl.multiple_of(i * TM, TM)
        yl = yl_ref[pl.ds(r0, TM), :]
        h = jnp.dot(yl, w1_ref[...], preferred_element_type=f32) + b1
        g = 0.5 * h * (1.0 + jnp.tanh(0.7978845608028654 * (h + 0.044715 * (h * h * h))))
        mo = jnp.dot(g.astype(bf16), w2_ref[...], preferred_element_type=f32)
        for s in range(TM // T):
            c = i * (TM // T) + s
            rr = pl.multiple_of(r0 + s * T, T)
            y = jnp.dot(Gm, yf_ref[c].astype(bf16), preferred_element_type=f32)
            xn = xn_ref[pl.ds(rr, T), :]
            res = x_ref[pl.ds(rr, T), :].astype(f32) + (y + xn * dsk) + (mo[s * T:(s + 1) * T] + b2)
            o_ref[pl.ds(rr, T), :] = res.astype(bf16)
        return carry
    if 'mlp' in parts:
        lax.fori_loop(0, L // TM, mlp_body, 0)
    else:
        o_ref[...] = jnp.zeros_like(o_ref)


def make(parts=('kmat', 'dftk', 'ln', 'conv', 'mlp')):
    def fn(A_u, A_A_re, A_A_im, A_B_re, A_B_im, A_C_re, A_C_im, A_log_dt, A_Dskip, B_x, B_w1, B_b1, B_w2, B_b2):
        x = A_u.reshape(L, D)
        Fc = jnp.asarray(_F_NP.astype(jnp.bfloat16)); Gc = jnp.asarray(_G_NP.astype(jnp.bfloat16))
        out = pl.pallas_call(
            functools.partial(kernel, parts=parts),
            out_shape=jax.ShapeDtypeStruct((L, D), bf16),
            scratch_shapes=[
                pltpu.VMEM((2, 8 * D, N), f32),
                pltpu.VMEM((2, 8 * D, N), f32),
                pltpu.VMEM((6, D, N), f32),
                pltpu.VMEM((NC * D, T), f32),
                pltpu.VMEM((NC, 256, D), f32),
                pltpu.VMEM((NC, 256, D), f32),
                pltpu.VMEM((NC, 256, D), bf16) if False else pltpu.VMEM((NC, 256, D), f32),
                pltpu.VMEM((L, D), f32),
                pltpu.VMEM((L, D), bf16),
            ],
            compiler_params=pltpu.CompilerParams(vmem_limit_bytes=110 * 1024 * 1024),
        )(x, A_A_re, A_A_im, A_B_re, A_B_im, A_C_re, A_C_im, A_log_dt, A_Dskip, B_w1, B_b1, B_w2, B_b2, Fc, Gc)
        return out.reshape(1, L, D)
    return jax.jit(fn)


_impl = make()


@jax.jit
def pallas_parallel_sum__ssm_conv_s4__mixer_channel_mlp__prompt_kernel(
    A_u, A_A_re, A_A_im, A_B_re, A_B_im, A_C_re, A_C_im, A_log_dt, A_Dskip,
    B_x, B_w1, B_b1, B_w2, B_b2,
):
    return _impl(A_u, A_A_re, A_A_im, A_B_re, A_B_im, A_C_re, A_C_im, A_log_dt, A_Dskip,
                 B_x, B_w1, B_b1, B_w2, B_b2)
```

```python
import numpy as np
import jax
import jax.numpy as jnp
from jax import lax
import jax.experimental.pallas as pl
import jax.experimental.pallas.tpu as pltpu

L, D, N, FF = 2048, 512, 128, 1792
T = 128
NC = L // T
S = D + 1
EPS = 1e-5
W = 256
NJ = FF // W

LN_UNR = 2
LN_ROWS = 32
P1_BODIES, P1_UNR, P1_TOK = 2, 4, 96
P3_ITERS = 4
OUT_UNR = 4

f32 = jnp.float32
bf16 = jnp.bfloat16
u32 = jnp.uint32
NT = (((1,), (1,)), ((), ()))


def _dft_consts():
    f = np.concatenate([np.arange(0, 128, 2), np.arange(1, 128, 2)])
    ang = (2 * np.pi * (f + 0.5) / 256)[:, None] * np.arange(128)[None, :]
    fwd = np.concatenate([np.cos(ang), -np.sin(ang)], 0)
    inv = np.concatenate([np.cos(ang).T, -np.sin(ang).T], 1) / 128.0
    return fwd.astype(np.float32), inv.astype(np.float32)


_F_NP, _G_NP = _dft_consts()


def _cmul(ar, ai, br, bi):
    return ar * br - ai * bi, ar * bi + ai * br


def _csq(ar, ai):
    return ar * ar - ai * ai, 2.0 * (ar * ai)


def _sincos(x):
    kf = jnp.round(x * 0.6366197723675814)
    r = ((x - kf * 1.5703125) - kf * 4.837512969970703125e-4) - kf * 7.54978995489188e-8
    z = r * r
    sp = r + r * z * ((-1.9515295891e-4 * z + 8.3321608736e-3) * z - 1.6666654611e-1)
    cp = (1.0 - 0.5 * z) + z * z * (
        (2.443315711809948e-5 * z - 1.388731625493765e-3) * z + 4.166664568298827e-2)
    q = kf.astype(jnp.int32)
    swap = (q & 1) == 1
    s_ = jnp.where(swap, cp, sp)
    c_ = jnp.where(swap, sp, cp)

    def flip(v, m):
        return pltpu.bitcast(pltpu.bitcast(v, jnp.int32) ^ m, f32)
    return flip(s_, (q & 2) << 30), flip(c_, ((q + 1) & 2) << 30)


def _zero_like_after(tok, z_ref):
    return pltpu.bitcast(pltpu.bitcast(tok, jnp.int32) & z_ref[...], f32)


def _kernel(x_hbm, are_hbm, aim_hbm, bre_hbm, bim_hbm, cre_hbm, cim_hbm, ldt_hbm, dsk_hbm,
            w1_hbm, b1_hbm, w2_hbm, b2_hbm, F_hbm, G_hbm,
            o_hbm,
            x_ref, par_ref, ldt_ref, dsk_ref, w1_ref, b1_ref, w2_ref, b2_ref, F_ref, G_ref, ob_ref,
            pf_ref, pc_ref, m_ref, kt_ref, kf_ref, uf_ref, yf_ref, acc_ref, yl_ref, xb_ref,
            cb_ref, z_ref, dtc_ref, sems, osem):
    cps = {}

    def start(name, src, dst, k):
        c = pltpu.make_async_copy(src, dst, sems.at[k])
        c.start()
        cps[name] = c

    start('ldt', ldt_hbm, ldt_ref, 0)
    for k, p in enumerate([are_hbm, aim_hbm, bre_hbm, bim_hbm, cre_hbm, cim_hbm]):
        start(('p', k), p, par_ref.at[k], 1 + k)
    start('F', F_hbm, F_ref, 7)
    start('x', x_hbm, x_ref, 8)
    start('dsk', dsk_hbm, dsk_ref, 9)
    start('b1', b1_hbm, b1_ref, 10)
    start('b2', b2_hbm, b2_ref, 11)
    start('G', G_hbm, G_ref, 12)
    for t in range(FF // 128):
        start(('w1', t), w1_hbm.at[:, pl.ds(t * 128, 128)], w1_ref.at[t], 13 + t)
    for t in range(D // 128):
        start(('w2', t), w2_hbm.at[:, pl.ds(t * 128, 128)], w2_ref.at[t], 27 + t)

    cps['ldt'].wait()
    for k in range(6):
        cps[('p', k)].wait()
    dt_row = jnp.exp(ldt_ref[...].astype(f32)).astype(bf16).astype(f32).reshape(1, D)
    dtc_ref[...] = jnp.broadcast_to(dt_row, (128, D)).T
    GC = 64
    NG = D // GC

    def a1_loop(builtin):
        def body(g, carry):
            rw = pl.ds(pl.multiple_of(g * GC, GC), GC)
            dt = dtc_ref[rw, :]
            e = jnp.exp(dt * par_ref[0, rw, :].astype(f32))
            th = dt * par_ref[1, rw, :].astype(f32)
            if builtin:
                sn, cs = jnp.sin(th), jnp.cos(th)
            else:
                sn, cs = _sincos(th)
            m_ref[0, rw, :] = e * cs
            m_ref[1, rw, :] = e * sn
            return carry
        lax.fori_loop(0, NG, body, 0)

    small = jnp.max(jnp.abs(dtc_ref[...] * par_ref[1].astype(f32))) <= 8192.0

    @pl.when(small)
    def _():
        a1_loop(False)

    @pl.when(jnp.logical_not(small))
    def _():
        a1_loop(True)

    for g in range(NG):
        r0 = g * GC
        rw = pl.ds(r0, GC)
        dt = dtc_ref[rw, :]
        a1 = (m_ref[0, rw, :], m_ref[1, rw, :])
        p = a1
        pf_ref[0, rw, :] = jnp.ones((GC, N), f32)
        pf_ref[1, rw, :] = jnp.zeros((GC, N), f32)
        for i in range(1, 8):
            pf_ref[0, pl.ds(i * S + r0, GC), :] = p[0]
            pf_ref[1, pl.ds(i * S + r0, GC), :] = p[1]
            p = _cmul(p[0], p[1], a1[0], a1[1])
        a8 = p
        a64 = _csq(*_csq(*_csq(*a8)))
        a128 = _csq(*a64)
        a1024 = _csq(*_csq(*_csq(*a128)))
        m_ref[0, rw, :] = a8[0]
        m_ref[1, rw, :] = a8[1]
        m_ref[2, rw, :] = a64[0]
        m_ref[3, rw, :] = -a64[1]
        m_ref[4, rw, :] = a1024[0]
        m_ref[5, rw, :] = -a1024[1]
        q = _cmul(par_ref[4, rw, :].astype(f32), par_ref[5, rw, :].astype(f32),
                  dt * par_ref[2, rw, :].astype(f32), dt * par_ref[3, rw, :].astype(f32))
        for i in range(8):
            pc_ref[0, pl.ds(i * S + r0, GC), :] = q[0]
            pc_ref[1, pl.ds(i * S + r0, GC), :] = -q[1]
            if i < 7:
                q = _cmul(q[0], q[1], a128[0], a128[1])

    lo = lax.broadcasted_iota(jnp.int32, (16, 128), 1) < 64
    H = D // 2

    def chan(d):
        def bc(k):
            return jnp.broadcast_to(m_ref[k, pl.ds(d, 1), :], (8, N))
        fr = pf_ref[0, pl.ds(d, 8, stride=S), :]
        fi = pf_ref[1, pl.ds(d, 8, stride=S), :]
        m8r, m8i = bc(0), bc(1)
        frs, fis = [fr], [fi]
        for _ in range(7):
            fr, fi = _cmul(fr, fi, m8r, m8i)
            frs.append(fr)
            fis.append(fi)
        c0 = (pc_ref[0, pl.ds(d, 8, stride=S), :], pc_ref[1, pl.ds(d, 8, stride=S), :])
        m64 = (bc(2), bc(3))
        m1k = (bc(4), bc(5))
        c1 = _cmul(*c0, *m1k)
        c2 = _cmul(*c0, *m64)
        c3 = _cmul(*c2, *m1k)
        return frs, fis, [c0[0], c1[0], c2[0], c3[0]], [c0[1], c1[1], c2[1], c3[1]]

    def kpair(p):
        fa = chan(p)
        fb = chan(p + H)

        def cat(a, b):
            return jnp.concatenate(a + b, 0)
        lhs = jnp.concatenate([cat(fa[2], fb[2]), cat(fa[3], fb[3])], 1).astype(bf16)
        rhs = jnp.concatenate([cat(fa[0], fb[0]), cat(fa[1], fb[1])], 1).astype(bf16)
        out = lax.dot_general(lhs, rhs, NT, preferred_element_type=f32)
        ka = jnp.where(lo, out[0:16], pltpu.roll(out[16:32], 64, 1))
        kb = jnp.where(lo, pltpu.roll(out[32:48], 64, 1), out[48:64])
        kt_ref[pl.ds(p, 16, stride=S), :] = ka
        kt_ref[pl.ds(p + H, 16, stride=S), :] = kb

    cps['F'].wait()
    cps['x'].wait()
    cps['dsk'].wait()
    cps['b2'].wait()
    cb_ref[0:8, 0:D] = jnp.broadcast_to(dsk_ref[...].astype(f32).reshape(1, D), (8, D))
    cb_ref[8:16, 0:D] = jnp.broadcast_to(b2_ref[...].astype(f32).reshape(1, D), (8, D))
    z_ref[...] = jnp.zeros_like(z_ref)
    RG = LN_ROWS

    def ln_rows(r0):
        x = x_ref[pl.ds(r0, RG), :].astype(f32)
        m = jnp.mean(x, axis=-1, keepdims=True)
        xc = x - m
        v = jnp.mean(xc * xc, axis=-1, keepdims=True)
        rs = lax.rsqrt(v + EPS)
        xn = xc * rs
        yl = xc * (rs * lax.rsqrt(v * rs * rs + EPS))
        h0 = pl.multiple_of(r0 // 2, RG // 2)
        yl_ref[pl.ds(h0, RG // 2), :] = pltpu.bitcast(yl.astype(bf16), u32)
        xb_ref[pl.ds(h0, RG // 2), :] = pltpu.bitcast(xn.astype(bf16), u32)

    def xn_block(c):
        return pltpu.bitcast(xb_ref[pl.ds(pl.multiple_of(c * (T // 2), T // 2), T // 2), :], bf16)

    def dftu_block(c):
        uf_ref[c] = jnp.dot(F_ref[...], xn_block(c), preferred_element_type=f32)

    def ln_body(i, carry):
        ip = jnp.maximum(i - 1, 0)
        for u in range(LN_UNR):
            dftu_block(ip * LN_UNR + u)
        for u in range(LN_UNR):
            r0 = pl.multiple_of((i * LN_UNR + u) * T, T)
            for g in range(T // RG):
                ln_rows(pl.multiple_of(r0 + g * RG, RG))
        return carry

    xb_ref[0:LN_UNR * T // 2, :] = jnp.zeros((LN_UNR * T // 2, D), u32)
    lax.fori_loop(0, NC // LN_UNR, ln_body, 0)
    for u in range(LN_UNR):
        dftu_block(NC - LN_UNR + u)

    cps['b1'].wait()
    for t in range(FF // 128):
        cps[('w1', t)].wait()
    for t in range(D // 128):
        cps[('w2', t)].wait()
    cps['G'].wait()
    cb_ref[16:24, :] = jnp.broadcast_to(b1_ref[...].astype(f32).reshape(1, FF), (8, FF))

    def w1_tile(t):
        return pltpu.bitcast(w1_ref.bitcast(u32)[t], bf16)

    def w2_tile(q, c0):
        return pltpu.bitcast(w2_ref.bitcast(u32)[q, c0 // 2:(c0 + W) // 2, :], bf16)

    def mlp_piece(r0, n, extra=None):
        yl = pltpu.bitcast(yl_ref[pl.ds(pl.multiple_of(r0 // 2, 8), n // 2), :], bf16)
        for j in range(NJ):
            c0 = j * W
            h = jnp.concatenate(
                [jnp.dot(yl, w1_tile(2 * j + q), preferred_element_type=f32) for q in range(2)], 1)
            h = h + cb_ref[16:17, c0:c0 + W]
            th = jnp.tanh(h * (0.7978845608028654 + (0.7978845608028654 * 0.044715) * (h * h)))
            g = (h + h * th).astype(bf16)
            if extra is not None:
                extra(2 * j)
            p = jnp.concatenate(
                [jnp.dot(g, w2_tile(q, c0), preferred_element_type=f32) for q in range(4)], 1)
            acc_ref[pl.ds(r0, n), :] = p if j == 0 else acc_ref[pl.ds(r0, n), :] + p
            if extra is not None:
                extra(2 * j + 1)

    PP = H // (P1_BODIES * P1_UNR)

    def p1_body(i, carry):
        for u in range(P1_UNR):
            it = i * P1_UNR + u

            def extra(k, it=it):
                ng = PP // 2
                for q in range(k * ng // (2 * NJ) * 2, (k + 1) * ng // (2 * NJ) * 2):
                    kpair(it * PP + q)
            mlp_piece(pl.multiple_of(it * P1_TOK, 16), P1_TOK, extra)
        return carry
    lax.fori_loop(0, P1_BODIES, p1_body, 0)
    tok0 = P1_BODIES * P1_UNR * P1_TOK

    def dftk_body(dt_, carry):
        d0 = pl.multiple_of(dt_ * 128, 128)
        prev = [None, None]
        for j in range(NC):
            kb = kt_ref[pl.ds(j * S + d0, 128), :].astype(bf16)
            for hf in range(2):
                fh = jnp.concatenate([F_ref[hf * 64:hf * 64 + 64, :],
                                      F_ref[128 + hf * 64:128 + hf * 64 + 64, :]], 0)
                cur = lax.dot_general(fh, kb, NT, preferred_element_type=f32)
                if j == 0:
                    re, im = cur[0:64], cur[64:128]
                elif hf == 0:
                    re, im = cur[0:64] - prev[0][64:128], cur[64:128] + prev[0][0:64]
                else:
                    re, im = cur[0:64] + prev[1][64:128], cur[64:128] - prev[1][0:64]
                kf_ref[j, hf * 64:hf * 64 + 64, pl.ds(d0, 128)] = re
                kf_ref[j, 128 + hf * 64:128 + hf * 64 + 64, pl.ds(d0, 128)] = im
                prev[hf] = cur
        return carry
    lax.fori_loop(0, D // 128, dftk_body, 0)

    TK3 = (L - tok0) // P3_ITERS
    PQ = 64 // P3_ITERS

    def conv_chain(it):
        tok = None
        for u in range(PQ):
            pos = it * PQ + u
            r = pl.multiple_of((pos // 4) * 8, 8)
            l0 = pl.multiple_of((pos % 4) * 128, 128)

            def ld(ref, i):
                return (ref[i, pl.ds(r, 8), pl.ds(l0, 128)],
                        ref[i, pl.ds(r + 128, 8), pl.ds(l0, 128)])
            for c in range(NC):
                ar = ai = None if tok is None else _zero_like_after(tok, z_ref)
                for j in range(c + 1):
                    ur, ui = ld(uf_ref, c - j)
                    kr, ki = ld(kf_ref, j)
                    if ar is None:
                        ar = ur * kr - ui * ki
                        ai = ur * ki + ui * kr
                    else:
                        ar = (ar + ur * kr) - ui * ki
                        ai = (ai + ur * ki) + ui * kr
                yf_ref[c, pl.ds(r, 8), pl.ds(l0, 128)] = ar
                yf_ref[c, pl.ds(r + 128, 8), pl.ds(l0, 128)] = ai
                tok = ai

    def p3_body(it, carry):
        mlp_piece(pl.multiple_of(tok0 + it * TK3, 16), TK3)
        conv_chain(it)
        return carry
    lax.fori_loop(0, P3_ITERS, p3_body, 0)

    def out_copy(c):
        r0 = pl.multiple_of(c * T, T)
        return pltpu.make_async_copy(ob_ref.at[pl.ds(r0, T)], o_hbm.at[pl.ds(r0, T)], osem)

    def p4_body(i, carry):
        for u in range(OUT_UNR):
            c = i * OUT_UNR + u
            r0 = pl.multiple_of(c * T, T)
            y = jnp.dot(G_ref[...], yf_ref[c].astype(bf16), preferred_element_type=f32)
            xn = xn_block(c).astype(f32)
            xx = x_ref[pl.ds(r0, T), :].astype(f32)
            res = ((xx + (y + xn * cb_ref[0:1, 0:D]))
                   + (0.5 * acc_ref[pl.ds(r0, T), :] + cb_ref[8:9, 0:D]))
            ob_ref[pl.ds(r0, T), :] = res.astype(bf16)
            out_copy(c).start()
        return carry
    lax.fori_loop(0, NC // OUT_UNR, p4_body, 0)
    for c in range(NC):
        out_copy(c).wait()


@jax.jit
def pallas_parallel_sum__ssm_conv_s4__mixer_channel_mlp__prompt_kernel(
    A_u: jax.Array,
    A_A_re: jax.Array,
    A_A_im: jax.Array,
    A_B_re: jax.Array,
    A_B_im: jax.Array,
    A_C_re: jax.Array,
    A_C_im: jax.Array,
    A_log_dt: jax.Array,
    A_Dskip: jax.Array,
    B_x: jax.Array,
    B_w1: jax.Array,
    B_b1: jax.Array,
    B_w2: jax.Array,
    B_b2: jax.Array,
):
    del B_x
    hbm = pl.BlockSpec(memory_space=pl.ANY)
    out = pl.pallas_call(
        _kernel,
        out_shape=jax.ShapeDtypeStruct((L, D), bf16),
        in_specs=[hbm] * 15,
        out_specs=hbm,
        scratch_shapes=[
            pltpu.VMEM((L, D), bf16),
            pltpu.VMEM((6, D, N), bf16),
            pltpu.VMEM((D,), bf16),
            pltpu.VMEM((D,), bf16),
            pltpu.VMEM((FF // 128, D, 128), bf16),
            pltpu.VMEM((FF,), bf16),
            pltpu.VMEM((D // 128, FF, 128), bf16),
            pltpu.VMEM((D,), bf16),
            pltpu.VMEM((256, T), bf16),
            pltpu.VMEM((T, 256), bf16),
            pltpu.VMEM((L, D), bf16),
            pltpu.VMEM((2, 8 * S, N), f32),
            pltpu.VMEM((2, 8 * S, N), f32),
            pltpu.VMEM((6, D, N), f32),
            pltpu.VMEM((NC * S, T), f32),
            pltpu.VMEM((NC, 256, D), f32),
            pltpu.VMEM((NC, 256, D), f32),
            pltpu.VMEM((NC, 256, D), f32),
            pltpu.VMEM((L, D), f32),
            pltpu.VMEM((L // 2, D), u32),
            pltpu.VMEM((L // 2, D), u32),
            pltpu.VMEM((24, FF), f32),
            pltpu.VMEM((8, 128), jnp.int32),
            pltpu.VMEM((D, N), f32),
            pltpu.SemaphoreType.DMA((31,)),
            pltpu.SemaphoreType.DMA,
        ],
        compiler_params=pltpu.CompilerParams(vmem_limit_bytes=110 * 1024 * 1024),
    )(A_u.reshape(L, D), A_A_re, A_A_im, A_B_re, A_B_im, A_C_re, A_C_im, A_log_dt, A_Dskip,
      B_w1, B_b1, B_w2, B_b2, _F_NP.astype(bf16), _G_NP.astype(bf16))
    return out.reshape(1, L, D)
```

```python
import numpy as np
import jax
import jax.numpy as jnp
from jax import lax
import jax.experimental.pallas as pl
import jax.experimental.pallas.tpu as pltpu

L, D, N, FF = 2048, 512, 128, 1792
T = 128
NC = L // T
S = D + 1
EPS = 1e-5
W = 256
NJ = FF // W

LN_UNR = 2
LN_ROWS = 32
P1_PIECES, P1_TOK = 8, 96
P3_ITERS = 4
OUT_UNR = 8

f32 = jnp.float32
bf16 = jnp.bfloat16
u32 = jnp.uint32
NT = (((1,), (1,)), ((), ()))


def _dft_consts():
    f = np.concatenate([np.arange(0, 128, 2), np.arange(1, 128, 2)])
    ang = (2 * np.pi * (f + 0.5) / 256)[:, None] * np.arange(128)[None, :]
    fwd = np.concatenate([np.cos(ang), -np.sin(ang)], 0)
    inv = np.concatenate([np.cos(ang).T, -np.sin(ang).T], 1) / 128.0
    return fwd.astype(np.float32), inv.astype(np.float32)


_F_NP, _G_NP = _dft_consts()


def _cmul(ar, ai, br, bi):
    return ar * br - ai * bi, ar * bi + ai * br


def _csq(ar, ai):
    return ar * ar - ai * ai, 2.0 * (ar * ai)


def _sincos(x):
    kf = jnp.round(x * 0.6366197723675814)
    r = ((x - kf * 1.5703125) - kf * 4.837512969970703125e-4) - kf * 7.54978995489188e-8
    z = r * r
    sp = r + r * z * ((-1.9515295891e-4 * z + 8.3321608736e-3) * z - 1.6666654611e-1)
    cp = (1.0 - 0.5 * z) + z * z * (
        (2.443315711809948e-5 * z - 1.388731625493765e-3) * z + 4.166664568298827e-2)
    q = kf.astype(jnp.int32)
    swap = (q & 1) == 1
    s_ = jnp.where(swap, cp, sp)
    c_ = jnp.where(swap, sp, cp)

    def flip(v, m):
        return pltpu.bitcast(pltpu.bitcast(v, jnp.int32) ^ m, f32)
    return flip(s_, (q & 2) << 30), flip(c_, ((q + 1) & 2) << 30)


def _zero_like_after(tok, z_ref):
    return pltpu.bitcast(pltpu.bitcast(tok, jnp.int32) & z_ref[...], f32)


def _kernel(x_hbm, are_hbm, aim_hbm, bre_hbm, bim_hbm, cre_hbm, cim_hbm, ldt_hbm, dsk_hbm,
            w1_hbm, b1_hbm, w2_hbm, b2_hbm, F_hbm, G_hbm,
            o_hbm,
            x_ref, par_ref, ldt_ref, dsk_ref, w1_ref, b1_ref, w2_ref, b2_ref, F_ref, G_ref, ob_ref,
            pf_ref, pc_ref, m_ref, kt_ref, kf_ref, uf_ref, yf_ref, acc_ref, yl_ref, xb_ref,
            cb_ref, z_ref, dtc_ref, sems, osem):
    cps = {}

    def start(name, src, dst, k):
        c = pltpu.make_async_copy(src, dst, sems.at[k])
        c.start()
        cps[name] = c

    start('ldt', ldt_hbm, ldt_ref, 0)
    for k, p in enumerate([are_hbm, aim_hbm, bre_hbm, bim_hbm, cre_hbm, cim_hbm]):
        start(('p', k), p, par_ref.at[k], 1 + k)
    start('F', F_hbm, F_ref, 7)
    start('x', x_hbm, x_ref, 8)
    start('dsk', dsk_hbm, dsk_ref, 9)
    start('b1', b1_hbm, b1_ref, 10)
    start('b2', b2_hbm, b2_ref, 11)
    start('G', G_hbm, G_ref, 12)
    for t in range(FF // 128):
        start(('w1', t), w1_hbm.at[:, pl.ds(t * 128, 128)], w1_ref.at[t], 13 + t)
    for t in range(D // 128):
        start(('w2', t), w2_hbm.at[:, pl.ds(t * 128, 128)], w2_ref.at[t], 27 + t)

    cps['ldt'].wait()
    for k in range(6):
        cps[('p', k)].wait()
    dt_row = jnp.exp(ldt_ref[...].astype(f32)).astype(bf16).astype(f32).reshape(1, D)
    dtc_ref[...] = jnp.broadcast_to(dt_row, (128, D)).T
    GC = 64
    NG = D // GC

    def a1_loop(builtin):
        def body(g, carry):
            rw = pl.ds(pl.multiple_of(g * GC, GC), GC)
            dt = dtc_ref[rw, :]
            e = jnp.exp(dt * par_ref[0, rw, :].astype(f32))
            th = dt * par_ref[1, rw, :].astype(f32)
            if builtin:
                sn, cs = jnp.sin(th), jnp.cos(th)
            else:
                sn, cs = _sincos(th)
            m_ref[0, rw, :] = e * cs
            m_ref[1, rw, :] = e * sn
            return carry
        lax.fori_loop(0, NG, body, 0)

    small = jnp.max(jnp.abs(dtc_ref[...] * par_ref[1].astype(f32))) <= 8192.0

    @pl.when(small)
    def _():
        a1_loop(False)

    @pl.when(jnp.logical_not(small))
    def _():
        a1_loop(True)

    z_ref[...] = jnp.zeros_like(z_ref)
    GT = 32
    toks = []
    for g in range(D // GT):
        r0 = g * GT
        rw = pl.ds(r0, GT)
        dt = dtc_ref[rw, :]
        a1 = (m_ref[0, rw, :], m_ref[1, rw, :])
        if len(toks) >= 2:
            a1 = (jnp.concatenate([a1[0][0:8] + _zero_like_after(toks.pop(0), z_ref), a1[0][8:]], 0), a1[1])
        p = a1
        pf_ref[0, rw, :] = jnp.ones((GT, N), f32)
        pf_ref[1, rw, :] = jnp.zeros((GT, N), f32)
        for i in range(1, 8):
            pf_ref[0, pl.ds(i * S + r0, GT), :] = p[0]
            pf_ref[1, pl.ds(i * S + r0, GT), :] = p[1]
            p = _cmul(p[0], p[1], a1[0], a1[1])
        a8 = p
        a64 = _csq(*_csq(*_csq(*a8)))
        a128 = _csq(*a64)
        a1024 = _csq(*_csq(*_csq(*a128)))
        m_ref[0, rw, :] = a8[0]
        m_ref[1, rw, :] = a8[1]
        m_ref[2, rw, :] = a64[0]
        m_ref[3, rw, :] = -a64[1]
        m_ref[4, rw, :] = a1024[0]
        m_ref[5, rw, :] = -a1024[1]
        q = _cmul(par_ref[4, rw, :].astype(f32), par_ref[5, rw, :].astype(f32),
                  dt * par_ref[2, rw, :].astype(f32), dt * par_ref[3, rw, :].astype(f32))
        for i in range(8):
            pc_ref[0, pl.ds(i * S + r0, GT), :] = q[0]
            pc_ref[1, pl.ds(i * S + r0, GT), :] = -q[1]
            if i < 7:
                q = _cmul(q[0], q[1], a128[0], a128[1])
        toks.append(q[0][0:8])

    lo = lax.broadcasted_iota(jnp.int32, (16, 128), 1) < 64
    H = D // 2

    def chan(d):
        def bc(k):
            return jnp.broadcast_to(m_ref[k, pl.ds(d, 1), :], (8, N))
        fr = pf_ref[0, pl.ds(d, 8, stride=S), :]
        fi = pf_ref[1, pl.ds(d, 8, stride=S), :]
        m8r, m8i = bc(0), bc(1)
        frs, fis = [fr], [fi]
        for _ in range(7):
            fr, fi = _cmul(fr, fi, m8r, m8i)
            frs.append(fr)
            fis.append(fi)
        c0 = (pc_ref[0, pl.ds(d, 8, stride=S), :], pc_ref[1, pl.ds(d, 8, stride=S), :])
        m64 = (bc(2), bc(3))
        m1k = (bc(4), bc(5))
        c1 = _cmul(*c0, *m1k)
        c2 = _cmul(*c0, *m64)
        c3 = _cmul(*c2, *m1k)
        return frs, fis, [c0[0], c1[0], c2[0], c3[0]], [c0[1], c1[1], c2[1], c3[1]]

    def kpair(p):
        fa = chan(p)
        fb = chan(p + H)

        def cat(a, b):
            return jnp.concatenate(a + b, 0)
        lhs = jnp.concatenate([cat(fa[2], fb[2]), cat(fa[3], fb[3])], 1).astype(bf16)
        rhs = jnp.concatenate([cat(fa[0], fb[0]), cat(fa[1], fb[1])], 1).astype(bf16)
        out = lax.dot_general(lhs, rhs, NT, preferred_element_type=f32)
        ka = jnp.where(lo, out[0:16], pltpu.roll(out[16:32], 64, 1))
        kb = jnp.where(lo, pltpu.roll(out[32:48], 64, 1), out[48:64])
        kt_ref[pl.ds(p, 16, stride=S), :] = ka
        kt_ref[pl.ds(p + H, 16, stride=S), :] = kb

    cps['F'].wait()
    cps['x'].wait()
    cps['dsk'].wait()
    cps['b2'].wait()
    cb_ref[0:8, 0:D] = jnp.broadcast_to(dsk_ref[...].astype(f32).reshape(1, D), (8, D))
    cb_ref[8:16, 0:D] = jnp.broadcast_to(b2_ref[...].astype(f32).reshape(1, D), (8, D))
    RG = LN_ROWS

    def ln_rows(r0):
        x = x_ref[pl.ds(r0, RG), :].astype(f32)
        m = jnp.mean(x, axis=-1, keepdims=True)
        xc = x - m
        v = jnp.mean(xc * xc, axis=-1, keepdims=True)
        rs = lax.rsqrt(v + EPS)
        xn = xc * rs
        yl = xc * (rs * lax.rsqrt(v * rs * rs + EPS))
        h0 = pl.multiple_of(r0 // 2, RG // 2)
        yl_ref[pl.ds(h0, RG // 2), :] = pltpu.bitcast(yl.astype(bf16), u32)
        xb_ref[pl.ds(h0, RG // 2), :] = pltpu.bitcast(xn.astype(bf16), u32)

    def xn_block(c):
        return pltpu.bitcast(xb_ref[pl.ds(pl.multiple_of(c * (T // 2), T // 2), T // 2), :], bf16)

    def dftu_block(c):
        uf_ref[c] = jnp.dot(F_ref[...], xn_block(c), preferred_element_type=f32)

    def ln_body(i, carry):
        ip = jnp.maximum(i - 1, 0)
        for u in range(LN_UNR):
            dftu_block(ip * LN_UNR + u)
        for u in range(LN_UNR):
            r0 = pl.multiple_of((i * LN_UNR + u) * T, T)
            for g in range(T // RG):
                ln_rows(pl.multiple_of(r0 + g * RG, RG))
        return carry

    xb_ref[0:LN_UNR * T // 2, :] = jnp.zeros((LN_UNR * T // 2, D), u32)
    lax.fori_loop(0, NC // LN_UNR, ln_body, 0)
    for u in range(LN_UNR):
        dftu_block(NC - LN_UNR + u)

    cps['b1'].wait()
    for t in range(FF // 128):
        cps[('w1', t)].wait()
    for t in range(D // 128):
        cps[('w2', t)].wait()
    cps['G'].wait()
    cb_ref[16:24, :] = jnp.broadcast_to(b1_ref[...].astype(f32).reshape(1, FF), (8, FF))

    def w1_tile(t):
        return pltpu.bitcast(w1_ref.bitcast(u32)[t], bf16)

    def w2_tile(q, c0):
        return pltpu.bitcast(w2_ref.bitcast(u32)[q, c0 // 2:(c0 + W) // 2, :], bf16)

    def mlp_piece(r0, n, extra=None):
        h0 = r0 // 2 if isinstance(r0, int) else pl.multiple_of(r0 // 2, 8)
        yl = pltpu.bitcast(yl_ref[pl.ds(h0, n // 2), :], bf16)
        for j in range(NJ):
            c0 = j * W
            h = jnp.concatenate(
                [jnp.dot(yl, w1_tile(2 * j + q), preferred_element_type=f32) for q in range(2)], 1)
            h = h + cb_ref[16:17, c0:c0 + W]
            th = jnp.tanh(h * (0.7978845608028654 + (0.7978845608028654 * 0.044715) * (h * h)))
            g = (h + h * th).astype(bf16)
            if extra is not None:
                extra(2 * j)
            p = jnp.concatenate(
                [jnp.dot(g, w2_tile(q, c0), preferred_element_type=f32) for q in range(4)], 1)
            acc_ref[pl.ds(r0, n), :] = p if j == 0 else acc_ref[pl.ds(r0, n), :] + p
            if extra is not None:
                extra(2 * j + 1)

    PP = H // P1_PIECES
    for it in range(P1_PIECES):
        def extra(k, it=it):
            ng = PP // 2
            for q in range(k * ng // (2 * NJ) * 2, (k + 1) * ng // (2 * NJ) * 2):
                kpair(it * PP + q)
        mlp_piece(it * P1_TOK, P1_TOK, extra)
    tok0 = P1_PIECES * P1_TOK

    for d0 in range(0, D, 128):
        prev = [None, None]
        for j in range(NC):
            kb = kt_ref[pl.ds(j * S + d0, 128), :].astype(bf16)
            for hf in range(2):
                fh = jnp.concatenate([F_ref[hf * 64:hf * 64 + 64, :],
                                      F_ref[128 + hf * 64:128 + hf * 64 + 64, :]], 0)
                cur = lax.dot_general(fh, kb, NT, preferred_element_type=f32)
                if j == 0:
                    re, im = cur[0:64], cur[64:128]
                elif hf == 0:
                    re, im = cur[0:64] - prev[0][64:128], cur[64:128] + prev[0][0:64]
                else:
                    re, im = cur[0:64] + prev[1][64:128], cur[64:128] - prev[1][0:64]
                kf_ref[j, hf * 64:hf * 64 + 64, pl.ds(d0, 128)] = re
                kf_ref[j, 128 + hf * 64:128 + hf * 64 + 64, pl.ds(d0, 128)] = im
                prev[hf] = cur

    TK3 = (L - tok0) // P3_ITERS
    PQ = 64 // P3_ITERS

    def conv_chain(it):
        tok = None
        nmac = 0
        for u in range(PQ):
            pos = it * PQ + u
            r = pl.multiple_of((pos // 4) * 8, 8)
            l0 = pl.multiple_of((pos % 4) * 128, 128)

            def ld(ref, i):
                return (ref[i, pl.ds(r, 8), pl.ds(l0, 128)],
                        ref[i, pl.ds(r + 128, 8), pl.ds(l0, 128)])
            for c in range(NC):
                ar = ai = None if tok is None else _zero_like_after(tok, z_ref)
                for j in range(c + 1):
                    ur, ui = ld(uf_ref, c - j)
                    kr, ki = ld(kf_ref, j)
                    if ar is None:
                        ar = ur * kr - ui * ki
                        ai = ur * ki + ui * kr
                    elif (nmac * 5) % 6 < 5:
                        ar = (ar + ur * kr) - ui * ki
                        ai = (ai + ur * ki) + ui * kr
                    else:
                        ar = ar + (ur * kr - ui * ki)
                        ai = ai + (ur * ki + ui * kr)
                    nmac += 1
                yf_ref[c, pl.ds(r, 8), pl.ds(l0, 128)] = ar
                yf_ref[c, pl.ds(r + 128, 8), pl.ds(l0, 128)] = ai
                tok = ai

    def p3_body(it, carry):
        mlp_piece(pl.multiple_of(tok0 + it * TK3, 16), TK3)
        conv_chain(it)
        return carry
    lax.fori_loop(0, P3_ITERS, p3_body, 0)

    def out_copy(c):
        r0 = pl.multiple_of(c * T, T)
        return pltpu.make_async_copy(ob_ref.at[pl.ds(r0, T)], o_hbm.at[pl.ds(r0, T)], osem)

    def p4_body(i, carry):
        for u in range(OUT_UNR):
            c = i * OUT_UNR + u
            r0 = pl.multiple_of(c * T, T)
            y = jnp.dot(G_ref[...], yf_ref[c].astype(bf16), preferred_element_type=f32)
            xn = xn_block(c).astype(f32)
            xx = x_ref[pl.ds(r0, T), :].astype(f32)
            res = ((xx + (y + xn * cb_ref[0:1, 0:D]))
                   + (0.5 * acc_ref[pl.ds(r0, T), :] + cb_ref[8:9, 0:D]))
            ob_ref[pl.ds(r0, T), :] = res.astype(bf16)
            out_copy(c).start()
        return carry
    lax.fori_loop(0, NC // OUT_UNR, p4_body, 0)
    for c in range(NC):
        out_copy(c).wait()


@jax.jit
def pallas_parallel_sum__ssm_conv_s4__mixer_channel_mlp__prompt_kernel(
    A_u: jax.Array,
    A_A_re: jax.Array,
    A_A_im: jax.Array,
    A_B_re: jax.Array,
    A_B_im: jax.Array,
    A_C_re: jax.Array,
    A_C_im: jax.Array,
    A_log_dt: jax.Array,
    A_Dskip: jax.Array,
    B_x: jax.Array,
    B_w1: jax.Array,
    B_b1: jax.Array,
    B_w2: jax.Array,
    B_b2: jax.Array,
):
    del B_x
    hbm = pl.BlockSpec(memory_space=pl.ANY)
    out = pl.pallas_call(
        _kernel,
        out_shape=jax.ShapeDtypeStruct((L, D), bf16),
        in_specs=[hbm] * 15,
        out_specs=hbm,
        scratch_shapes=[
            pltpu.VMEM((L, D), bf16),
            pltpu.VMEM((6, D, N), bf16),
            pltpu.VMEM((D,), bf16),
            pltpu.VMEM((D,), bf16),
            pltpu.VMEM((FF // 128, D, 128), bf16),
            pltpu.VMEM((FF,), bf16),
            pltpu.VMEM((D // 128, FF, 128), bf16),
            pltpu.VMEM((D,), bf16),
            pltpu.VMEM((256, T), bf16),
            pltpu.VMEM((T, 256), bf16),
            pltpu.VMEM((L, D), bf16),
            pltpu.VMEM((2, 8 * S, N), f32),
            pltpu.VMEM((2, 8 * S, N), f32),
            pltpu.VMEM((6, D, N), f32),
            pltpu.VMEM((NC * S, T), f32),
            pltpu.VMEM((NC, 256, D), f32),
            pltpu.VMEM((NC, 256, D), f32),
            pltpu.VMEM((NC, 256, D), f32),
            pltpu.VMEM((L, D), f32),
            pltpu.VMEM((L // 2, D), u32),
            pltpu.VMEM((L // 2, D), u32),
            pltpu.VMEM((24, FF), f32),
            pltpu.VMEM((8, 128), jnp.int32),
            pltpu.VMEM((D, N), f32),
            pltpu.SemaphoreType.DMA((31,)),
            pltpu.SemaphoreType.DMA,
        ],
        compiler_params=pltpu.CompilerParams(vmem_limit_bytes=110 * 1024 * 1024),
    )(A_u.reshape(L, D), A_A_re, A_A_im, A_B_re, A_B_im, A_C_re, A_C_im, A_log_dt, A_Dskip,
      B_w1, B_b1, B_w2, B_b2, _F_NP.astype(bf16), _G_NP.astype(bf16))
    return out.reshape(1, L, D)
```

```python
import numpy as np
import jax
import jax.numpy as jnp
from jax import lax
import jax.experimental.pallas as pl
import jax.experimental.pallas.tpu as pltpu

L, D, N, FF = 2048, 512, 128, 1792
T = 128
NC = L // T
S = D + 1
EPS = 1e-5
W = 256
NJ = FF // W

LN_ROWS = 32
P1_PIECES, P1_TOK = 8, 96
C0 = 6
K0 = 64
P3_ITERS = 2
OUT_UNR = 8

f32 = jnp.float32
bf16 = jnp.bfloat16
u32 = jnp.uint32
NT = (((1,), (1,)), ((), ()))


def _dft_consts():
    f = np.concatenate([np.arange(0, 128, 2), np.arange(1, 128, 2)])
    ang = (2 * np.pi * (f + 0.5) / 256)[:, None] * np.arange(128)[None, :]
    fwd = np.concatenate([np.cos(ang), -np.sin(ang)], 0)
    inv = np.concatenate([np.cos(ang).T, -np.sin(ang).T], 1) / 128.0
    return fwd.astype(np.float32), inv.astype(np.float32)


_F_NP, _G_NP = _dft_consts()


def _cmul(ar, ai, br, bi):
    return ar * br - ai * bi, ar * bi + ai * br


def _csq(ar, ai):
    return ar * ar - ai * ai, 2.0 * (ar * ai)


def _sincos(x):
    kf = jnp.round(x * 0.6366197723675814)
    r = ((x - kf * 1.5703125) - kf * 4.837512969970703125e-4) - kf * 7.54978995489188e-8
    z = r * r
    sp = r + r * z * ((-1.9515295891e-4 * z + 8.3321608736e-3) * z - 1.6666654611e-1)
    cp = (1.0 - 0.5 * z) + z * z * (
        (2.443315711809948e-5 * z - 1.388731625493765e-3) * z + 4.166664568298827e-2)
    q = kf.astype(jnp.int32)
    swap = (q & 1) == 1
    s_ = jnp.where(swap, cp, sp)
    c_ = jnp.where(swap, sp, cp)

    def flip(v, m):
        return pltpu.bitcast(pltpu.bitcast(v, jnp.int32) ^ m, f32)
    return flip(s_, (q & 2) << 30), flip(c_, ((q + 1) & 2) << 30)


def _zero_like_after(tok, z_ref):
    return pltpu.bitcast(pltpu.bitcast(tok, jnp.int32) & z_ref[...], f32)


def _kernel(x_hbm, are_hbm, aim_hbm, bre_hbm, bim_hbm, cre_hbm, cim_hbm, ldt_hbm, dsk_hbm,
            w1_hbm, b1_hbm, w2_hbm, b2_hbm, F_hbm, G_hbm,
            o_hbm,
            x_ref, par_ref, ldt_ref, dsk_ref, w1_ref, b1_ref, w2_ref, b2_ref, F_ref, G_ref, ob_ref,
            pf_ref, pc_ref, m_ref, kt_ref, kf_ref, uf_ref, yf_ref, acc_ref, yl_ref, xb_ref,
            cb_ref, z_ref, dtc_ref, sems, osem):
    cps = {}

    def start(name, src, dst, k):
        c = pltpu.make_async_copy(src, dst, sems.at[k])
        c.start()
        cps[name] = c

    start('ldt', ldt_hbm, ldt_ref, 0)
    for k, p in enumerate([are_hbm, aim_hbm, bre_hbm, bim_hbm, cre_hbm, cim_hbm]):
        start(('p', k), p, par_ref.at[k], 1 + k)
    start('F', F_hbm, F_ref, 7)
    start('x0', x_hbm.at[pl.ds(0, C0 * T)], x_ref.at[pl.ds(0, C0 * T)], 8)
    start('dsk', dsk_hbm, dsk_ref, 9)
    start('b1', b1_hbm, b1_ref, 10)
    start('b2', b2_hbm, b2_ref, 11)
    start('G', G_hbm, G_ref, 12)
    for t in range(FF // 128):
        start(('w1', t), w1_hbm.at[:, pl.ds(t * 128, 128)], w1_ref.at[t], 13 + t)
    for t in range(D // 128):
        start(('w2', t), w2_hbm.at[:, pl.ds(t * 128, 128)], w2_ref.at[t], 27 + t)
    start('x1', x_hbm.at[pl.ds(C0 * T, L - C0 * T)], x_ref.at[pl.ds(C0 * T, L - C0 * T)], 31)

    cps['ldt'].wait()
    cps[('p', 0)].wait()
    cps[('p', 1)].wait()
    dt_row = jnp.exp(ldt_ref[...].astype(f32)).astype(bf16).astype(f32).reshape(1, D)
    dtc_ref[...] = jnp.broadcast_to(dt_row, (128, D)).T
    GC = 64
    NG = D // GC

    def a1_loop(builtin):
        def body(g, carry):
            rw = pl.ds(pl.multiple_of(g * GC, GC), GC)
            dt = dtc_ref[rw, :]
            e = jnp.exp(dt * par_ref[0, rw, :].astype(f32))
            th = dt * par_ref[1, rw, :].astype(f32)
            if builtin:
                sn, cs = jnp.sin(th), jnp.cos(th)
            else:
                sn, cs = _sincos(th)
            m_ref[0, rw, :] = e * cs
            m_ref[1, rw, :] = e * sn
            return carry
        lax.fori_loop(0, NG, body, 0)

    small = jnp.max(jnp.abs(dtc_ref[...] * par_ref[1].astype(f32))) <= 8192.0

    @pl.when(small)
    def _():
        a1_loop(False)

    @pl.when(jnp.logical_not(small))
    def _():
        a1_loop(True)

    for k in range(2, 6):
        cps[('p', k)].wait()
    z_ref[...] = jnp.zeros_like(z_ref)
    GT = 32
    toks = []
    for g in range(D // GT):
        r0 = g * GT
        rw = pl.ds(r0, GT)
        dt = dtc_ref[rw, :]
        a1 = (m_ref[0, rw, :], m_ref[1, rw, :])
        if len(toks) >= 2:
            a1 = (jnp.concatenate([a1[0][0:8] + _zero_like_after(toks.pop(0), z_ref), a1[0][8:]], 0), a1[1])
        p = a1
        pf_ref[0, rw, :] = jnp.ones((GT, N), f32)
        pf_ref[1, rw, :] = jnp.zeros((GT, N), f32)
        for i in range(1, 8):
            pf_ref[0, pl.ds(i * S + r0, GT), :] = p[0]
            pf_ref[1, pl.ds(i * S + r0, GT), :] = p[1]
            p = _cmul(p[0], p[1], a1[0], a1[1])
        a8 = p
        a64 = _csq(*_csq(*_csq(*a8)))
        a128 = _csq(*a64)
        a1024 = _csq(*_csq(*_csq(*a128)))
        m_ref[0, rw, :] = a8[0]
        m_ref[1, rw, :] = a8[1]
        m_ref[2, rw, :] = a64[0]
        m_ref[3, rw, :] = -a64[1]
        m_ref[4, rw, :] = a1024[0]
        m_ref[5, rw, :] = -a1024[1]
        q = _cmul(par_ref[4, rw, :].astype(f32), par_ref[5, rw, :].astype(f32),
                  dt * par_ref[2, rw, :].astype(f32), dt * par_ref[3, rw, :].astype(f32))
        for i in range(8):
            pc_ref[0, pl.ds(i * S + r0, GT), :] = q[0]
            pc_ref[1, pl.ds(i * S + r0, GT), :] = -q[1]
            if i < 7:
                q = _cmul(q[0], q[1], a128[0], a128[1])
        toks.append(q[0][0:8])

    lo = lax.broadcasted_iota(jnp.int32, (16, 128), 1) < 64
    H = D // 2

    def chan(d):
        def bc(k):
            return jnp.broadcast_to(m_ref[k, pl.ds(d, 1), :], (8, N))
        fr = pf_ref[0, pl.ds(d, 8, stride=S), :]
        fi = pf_ref[1, pl.ds(d, 8, stride=S), :]
        m8r, m8i = bc(0), bc(1)
        frs, fis = [fr], [fi]
        for _ in range(7):
            fr, fi = _cmul(fr, fi, m8r, m8i)
            frs.append(fr)
            fis.append(fi)
        c0 = (pc_ref[0, pl.ds(d, 8, stride=S), :], pc_ref[1, pl.ds(d, 8, stride=S), :])
        m64 = (bc(2), bc(3))
        m1k = (bc(4), bc(5))
        c1 = _cmul(*c0, *m1k)
        c2 = _cmul(*c0, *m64)
        c3 = _cmul(*c2, *m1k)
        return frs, fis, [c0[0], c1[0], c2[0], c3[0]], [c0[1], c1[1], c2[1], c3[1]]

    def kpair(p):
        fa = chan(p)
        fb = chan(p + H)

        def cat(a, b):
            return jnp.concatenate(a + b, 0)
        lhs = jnp.concatenate([cat(fa[2], fb[2]), cat(fa[3], fb[3])], 1).astype(bf16)
        rhs = jnp.concatenate([cat(fa[0], fb[0]), cat(fa[1], fb[1])], 1).astype(bf16)
        out = lax.dot_general(lhs, rhs, NT, preferred_element_type=f32)
        ka = jnp.where(lo, out[0:16], pltpu.roll(out[16:32], 64, 1))
        kb = jnp.where(lo, pltpu.roll(out[32:48], 64, 1), out[48:64])
        kt_ref[pl.ds(p, 16, stride=S), :] = ka
        kt_ref[pl.ds(p + H, 16, stride=S), :] = kb

    cps['F'].wait()
    cps['x0'].wait()
    cps['dsk'].wait()
    cps['b2'].wait()
    cb_ref[0:8, 0:D] = jnp.broadcast_to(dsk_ref[...].astype(f32).reshape(1, D), (8, D))
    cb_ref[8:16, 0:D] = jnp.broadcast_to(b2_ref[...].astype(f32).reshape(1, D), (8, D))
    RG = LN_ROWS

    def ln_rows(r0):
        x = x_ref[pl.ds(r0, RG), :].astype(f32)
        m = jnp.mean(x, axis=-1, keepdims=True)
        xc = x - m
        v = jnp.mean(xc * xc, axis=-1, keepdims=True)
        rs = lax.rsqrt(v + EPS)
        xn = xc * rs
        yl = xc * (rs * lax.rsqrt(v * rs * rs + EPS))
        h0 = r0 // 2 if isinstance(r0, int) else pl.multiple_of(r0 // 2, RG // 2)
        yl_ref[pl.ds(h0, RG // 2), :] = pltpu.bitcast(yl.astype(bf16), u32)
        xb_ref[pl.ds(h0, RG // 2), :] = pltpu.bitcast(xn.astype(bf16), u32)

    def xn_block(c):
        h0 = c * (T // 2) if isinstance(c, int) else pl.multiple_of(c * (T // 2), T // 2)
        return pltpu.bitcast(xb_ref[pl.ds(h0, T // 2), :], bf16)

    def dftu_block(c):
        uf_ref[c] = jnp.dot(F_ref[...], xn_block(c), preferred_element_type=f32)

    for c in range(C0 + 1):
        if c > 0:
            dftu_block(c - 1)
        if c < C0:
            for g in range(T // RG):
                ln_rows(c * T + g * RG)
        for p in range(c * (K0 // 2) // (C0 + 1) * 2, (c + 1) * (K0 // 2) // (C0 + 1) * 2):
            kpair(p)

    cps['b1'].wait()
    for t in range(FF // 128):
        cps[('w1', t)].wait()
    for t in range(D // 128):
        cps[('w2', t)].wait()
    cps['G'].wait()
    cb_ref[16:24, :] = jnp.broadcast_to(b1_ref[...].astype(f32).reshape(1, FF), (8, FF))

    def w1_tile(t):
        return pltpu.bitcast(w1_ref.bitcast(u32)[t], bf16)

    def w2_tile(q, c0):
        return pltpu.bitcast(w2_ref.bitcast(u32)[q, c0 // 2:(c0 + W) // 2, :], bf16)

    def mlp_piece(r0, n, extra=None):
        h0 = r0 // 2 if isinstance(r0, int) else pl.multiple_of(r0 // 2, 8)
        yl = pltpu.bitcast(yl_ref[pl.ds(h0, n // 2), :], bf16)
        for j in range(NJ):
            c0 = j * W
            h = jnp.concatenate(
                [jnp.dot(yl, w1_tile(2 * j + q), preferred_element_type=f32) for q in range(2)], 1)
            h = h + cb_ref[16:17, c0:c0 + W]
            th = jnp.tanh(h * (0.7978845608028654 + (0.7978845608028654 * 0.044715) * (h * h)))
            g = (h + h * th).astype(bf16)
            if extra is not None:
                extra(2 * j)
            p = jnp.concatenate(
                [jnp.dot(g, w2_tile(q, c0), preferred_element_type=f32) for q in range(4)], 1)
            acc_ref[pl.ds(r0, n), :] = p if j == 0 else acc_ref[pl.ds(r0, n), :] + p
            if extra is not None:
                extra(2 * j + 1)

    PP = (H - K0) // P1_PIECES
    for it in range(P1_PIECES):
        def extra(k, it=it):
            ng = PP // 2
            for q in range(k * ng // (2 * NJ) * 2, (k + 1) * ng // (2 * NJ) * 2):
                kpair(K0 + it * PP + q)
        mlp_piece(it * P1_TOK, P1_TOK, extra)
    tok0 = P1_PIECES * P1_TOK

    cps['x1'].wait()
    n1 = NC - C0

    def ln1_step(k):
        for c in range(k * (n1 + 1) // 64, (k + 1) * (n1 + 1) // 64):
            if c > 0:
                dftu_block(C0 + c - 1)
            if c < n1:
                for g in range(T // RG):
                    ln_rows((C0 + c) * T + g * RG)

    for d0 in range(0, D, 128):
        prev = [None, None]
        for j in range(NC):
            kb = kt_ref[pl.ds(j * S + d0, 128), :].astype(bf16)
            for hf in range(2):
                fh = jnp.concatenate([F_ref[hf * 64:hf * 64 + 64, :],
                                      F_ref[128 + hf * 64:128 + hf * 64 + 64, :]], 0)
                cur = lax.dot_general(fh, kb, NT, preferred_element_type=f32)
                if j == 0:
                    re, im = cur[0:64], cur[64:128]
                elif hf == 0:
                    re, im = cur[0:64] - prev[0][64:128], cur[64:128] + prev[0][0:64]
                else:
                    re, im = cur[0:64] + prev[1][64:128], cur[64:128] - prev[1][0:64]
                kf_ref[j, hf * 64:hf * 64 + 64, pl.ds(d0, 128)] = re
                kf_ref[j, 128 + hf * 64:128 + hf * 64 + 64, pl.ds(d0, 128)] = im
                prev[hf] = cur
            ln1_step(d0 // 128 * NC + j)

    TK3 = (L - tok0) // P3_ITERS
    PQ = 64 // P3_ITERS

    def conv_chain(it):
        tok = None
        nmac = 0
        for u in range(PQ):
            pos = it * PQ + u
            r = pl.multiple_of((pos // 4) * 8, 8)
            l0 = pl.multiple_of((pos % 4) * 128, 128)

            def ld(ref, i):
                return (ref[i, pl.ds(r, 8), pl.ds(l0, 128)],
                        ref[i, pl.ds(r + 128, 8), pl.ds(l0, 128)])
            for c in range(NC):
                ar = ai = None if tok is None else _zero_like_after(tok, z_ref)
                for j in range(c + 1):
                    ur, ui = ld(uf_ref, c - j)
                    kr, ki = ld(kf_ref, j)
                    if ar is None:
                        ar = ur * kr - ui * ki
                        ai = ur * ki + ui * kr
                    elif (nmac * 5) % 6 < 5:
                        ar = (ar + ur * kr) - ui * ki
                        ai = (ai + ur * ki) + ui * kr
                    else:
                        ar = ar + (ur * kr - ui * ki)
                        ai = ai + (ur * ki + ui * kr)
                    nmac += 1
                yf_ref[c, pl.ds(r, 8), pl.ds(l0, 128)] = ar
                yf_ref[c, pl.ds(r + 128, 8), pl.ds(l0, 128)] = ai
                tok = ai

    def p3_body(it, carry):
        mlp_piece(pl.multiple_of(tok0 + it * TK3, 16), TK3)
        conv_chain(it)
        return carry
    lax.fori_loop(0, P3_ITERS, p3_body, 0)

    def out_copy(c):
        r0 = pl.multiple_of(c * T, T)
        return pltpu.make_async_copy(ob_ref.at[pl.ds(r0, T)], o_hbm.at[pl.ds(r0, T)], osem)

    def p4_body(i, carry):
        for u in range(OUT_UNR):
            c = i * OUT_UNR + u
            r0 = pl.multiple_of(c * T, T)
            y = jnp.dot(G_ref[...], yf_ref[c].astype(bf16), preferred_element_type=f32)
            xn = xn_block(c).astype(f32)
            xx = x_ref[pl.ds(r0, T), :].astype(f32)
            res = ((xx + (y + xn * cb_ref[0:1, 0:D]))
                   + (0.5 * acc_ref[pl.ds(r0, T), :] + cb_ref[8:9, 0:D]))
            ob_ref[pl.ds(r0, T), :] = res.astype(bf16)
            out_copy(c).start()
        return carry
    lax.fori_loop(0, NC // OUT_UNR, p4_body, 0)
    for c in range(NC):
        out_copy(c).wait()


@jax.jit
def pallas_parallel_sum__ssm_conv_s4__mixer_channel_mlp__prompt_kernel(
    A_u: jax.Array,
    A_A_re: jax.Array,
    A_A_im: jax.Array,
    A_B_re: jax.Array,
    A_B_im: jax.Array,
    A_C_re: jax.Array,
    A_C_im: jax.Array,
    A_log_dt: jax.Array,
    A_Dskip: jax.Array,
    B_x: jax.Array,
    B_w1: jax.Array,
    B_b1: jax.Array,
    B_w2: jax.Array,
    B_b2: jax.Array,
):
    del B_x
    hbm = pl.BlockSpec(memory_space=pl.ANY)
    out = pl.pallas_call(
        _kernel,
        out_shape=jax.ShapeDtypeStruct((L, D), bf16),
        in_specs=[hbm] * 15,
        out_specs=hbm,
        scratch_shapes=[
            pltpu.VMEM((L, D), bf16),
            pltpu.VMEM((6, D, N), bf16),
            pltpu.VMEM((D,), bf16),
            pltpu.VMEM((D,), bf16),
            pltpu.VMEM((FF // 128, D, 128), bf16),
            pltpu.VMEM((FF,), bf16),
            pltpu.VMEM((D // 128, FF, 128), bf16),
            pltpu.VMEM((D,), bf16),
            pltpu.VMEM((256, T), bf16),
            pltpu.VMEM((T, 256), bf16),
            pltpu.VMEM((L, D), bf16),
            pltpu.VMEM((2, 8 * S, N), f32),
            pltpu.VMEM((2, 8 * S, N), f32),
            pltpu.VMEM((6, D, N), f32),
            pltpu.VMEM((NC * S, T), f32),
            pltpu.VMEM((NC, 256, D), f32),
            pltpu.VMEM((NC, 256, D), f32),
            pltpu.VMEM((NC, 256, D), f32),
            pltpu.VMEM((L, D), f32),
            pltpu.VMEM((L // 2, D), u32),
            pltpu.VMEM((L // 2, D), u32),
            pltpu.VMEM((24, FF), f32),
            pltpu.VMEM((8, 128), jnp.int32),
            pltpu.VMEM((D, N), f32),
            pltpu.SemaphoreType.DMA((32,)),
            pltpu.SemaphoreType.DMA,
        ],
        compiler_params=pltpu.CompilerParams(vmem_limit_bytes=110 * 1024 * 1024),
    )(A_u.reshape(L, D), A_A_re, A_A_im, A_B_re, A_B_im, A_C_re, A_C_im, A_log_dt, A_Dskip,
      B_w1, B_b1, B_w2, B_b2, _F_NP.astype(bf16), _G_NP.astype(bf16))
    return out.reshape(1, L, D)
```
